```python
import os as _os
_os.environ.setdefault('JAX_PLATFORMS', 'cpu')
import jax
import jax.numpy as jnp

def _softmax(x, axis=-1):
    return jax.nn.softmax(x, axis=axis)

def _gelu(x):
    return jax.nn.gelu(x, approximate=True)

def _silu(x):
    return jax.nn.silu(x)

def _sigmoid(x):
    return jax.nn.sigmoid(x)

def _layernorm(x, axis=-1, eps=1e-05):
    m = jnp.mean(x, axis=axis, keepdims=True)
    v = jnp.var(x, axis=axis, keepdims=True)
    return (x - m) / jnp.sqrt(v + eps)

def _scatter_add(tgt, idx, src, axis=0):
    return tgt.at[idx].add(src)

def _segment_sum(src, seg, n):
    return jax.ops.segment_sum(src, seg, n)

class _Rng:

    def __init__(self, key):
        self._k = key

    def _next(self):
        self._k, sub = jax.random.split(self._k)
        return sub

    def normal(self, shape):
        return jax.random.normal(self._next(), shape, dtype=jnp.bfloat16)

    def randint(self, lo, hi, shape):
        return jax.random.randint(self._next(), shape, lo, hi, dtype=jnp.int32)

    def uniform(self, shape, lo=0.0, hi=1.0):
        return jax.random.uniform(self._next(), shape, jnp.bfloat16, lo, hi)

    def permutation(self, n):
        return jax.random.permutation(self._next(), n)
kernel_name = 'adaLN_cond__memory_aug_recurrent_mem_tr__moe_arch_mod__prompt'

def setup_inputs():
    _rng = _Rng(jax.random.key(int.from_bytes(__import__("os").urandom(4), "little")))
    _w = lambda a: (lambda t: t.astype(jnp.bfloat16) if jnp.issubdtype(t.dtype, jnp.floating) else t)(jnp.asarray(a))

    def _A_setup():
        B, S, Dm = (1, 2048, 448)
        H, Dh = (16, 256)
        M, seg = (8, 32)
        seg = min(seg, S)
        S = S // seg * seg
        return {'x': _w((lambda *s: _rng.normal(s) * 0.05)(B, S, Dm)), 'mem0': _w((lambda *s: _rng.normal(s) * 0.4)(B, M, Dm)), 'Wq': _w((lambda *s: _rng.normal(s) * 1.6)(Dm, H, Dh) * Dm ** (-0.5)), 'Wk': _w((lambda *s: _rng.normal(s) * 1.6)(Dm, H, Dh) * Dm ** (-0.5)), 'Wv': _w((lambda *s: _rng.normal(s) * 0.4)(Dm, H, Dh) * Dm ** (-0.5)), 'Wo': _w((lambda *s: _rng.normal(s) * 0.4)(H, Dh, Dm) * (H * Dh) ** (-0.5)), 'seg_len': seg}
    _A_in = _A_setup()

    def _B_setup():
        B, S, D, F, C = (1, 2048, 448, 1792, 1)
        return {'x': _w((lambda *s: _rng.normal(s) * 0.05)(B, S, D)), 'w_r': _w((lambda *s: _rng.normal(s) * 0.05)(D)), 'w_gate': _w((lambda *s: _rng.normal(s) * 0.05)(D, F)), 'w_up': _w((lambda *s: _rng.normal(s) * 0.05)(D, F)), 'w_down': _w((lambda *s: _rng.normal(s) * 0.05)(F, D))}
    _B_in = _B_setup()
    return {'A_x': _A_in['x'], 'A_mem0': _A_in['mem0'], 'A_Wq': _A_in['Wq'], 'A_Wk': _A_in['Wk'], 'A_Wv': _A_in['Wv'], 'A_Wo': _A_in['Wo'], 'A_seg_len': _A_in['seg_len'], 'B_x': _B_in['x'], 'B_w_r': _B_in['w_r'], 'B_w_gate': _B_in['w_gate'], 'B_w_up': _B_in['w_up'], 'B_w_down': _B_in['w_down'], 'c': _w((lambda *s: _rng.normal(s) * 0.05)(1, 448) * 8.0), 'w_mod': _w((lambda *s: _rng.normal(s) * 0.05)(448, 6 * 448) * 448 ** (-0.5) * 8.0)}

def reference(A_x, A_mem0, A_Wq, A_Wk, A_Wv, A_Wo, A_seg_len, B_x, B_w_r, B_w_gate, B_w_up, B_w_down, c, w_mod):

    def _A_ref(x, mem0, Wq, Wk, Wv, Wo, seg_len):
        B, S, Dm = x.shape
        H, Dh = (Wq.shape[1], Wq.shape[2])
        M = mem0.shape[1]
        scale = Dh ** (-0.5)
        n_seg = S // seg_len
        L = M + seg_len
        idx = jnp.arange(L)
        mask = (idx[:, None] < M) | (idx[:, None] >= idx[None, :])
        mem = mem0
        outs = []
        for s in range(n_seg):
            xs = x[:, s * seg_len:(s + 1) * seg_len, :].copy()
            h = jnp.concatenate([mem, xs], axis=1)
            q = jnp.einsum('btd,dhe->bhte', h, Wq)
            k = jnp.einsum('btd,dhe->bhte', h, Wk)
            v = jnp.einsum('btd,dhe->bhte', h, Wv)
            scores = jnp.einsum('bhqe,bhke->bhqk', q, k) * scale
            scores = jnp.where(mask[None, None], scores, -1000000000.0)
            p = _softmax(scores, axis=-1)
            o = jnp.einsum('bhqk,bhke->bhqe', p, v)
            o = jnp.einsum('bhte,hed->btd', o, Wo)
            mem = o[:, :M, :].copy()
            outs.append(o[:, M:, :])
        return jnp.concatenate(outs, axis=1)

    def _B_ref(x, w_r, w_gate, w_up, w_down):
        B, S, D = x.shape
        C = 1
        r = x @ w_r
        idx = jnp.argsort(-r, axis=-1)[:, :C]
        idx_e = jnp.repeat(idx.reshape(B, C, 1), D, axis=2)
        x_sel = jnp.take_along_axis(x, idx_e, axis=1)
        g = _silu(x_sel @ w_gate)
        u = x_sel @ w_up
        y = g * u @ w_down
        r_sel = _sigmoid(jnp.take_along_axis(r, idx, axis=1))
        y = y * r_sel.reshape(B, C, 1)
        b_off = (jnp.arange(B) * S).reshape(B, 1)
        flat_idx = (idx + b_off).reshape(B * C)
        zero = (x * 0.0).reshape(B * S, D)
        upd = _scatter_add(zero, flat_idx, y.reshape(B * C, D), axis=0)
        return x + upd.reshape(B, S, D)
    x = A_x
    mod = (_silu(c) @ w_mod).reshape(c.shape[0], 6, 1, -1)
    sa, ca, ga, sb, cb, gb = (mod[:, 0].copy(), mod[:, 1].copy(), mod[:, 2].copy(), mod[:, 3].copy(), mod[:, 4].copy(), mod[:, 5].copy())
    h = _layernorm(x, axis=-1) * (1 + ca) + sa
    x = x + ga * _A_ref(h, A_mem0, A_Wq, A_Wk, A_Wv, A_Wo, A_seg_len)
    h = _layernorm(x, axis=-1) * (1 + cb) + sb
    x = x + gb * _B_ref(h, B_w_r, B_w_gate, B_w_up, B_w_down)
    return x
```

```python
import functools

import jax
import jax.numpy as jnp
from jax import lax
import jax.experimental.pallas as pl
import jax.experimental.pallas.tpu as pltpu

F32 = jnp.float32
BF16 = jnp.bfloat16

S = 2048
D = 448
H = 16
DH = 256
M = 8
SEG = 32
NSEG = S // SEG
FF = 1792
DM = 384
DE = 512
PW = 896
NCH = 8
CW = 2 * PW
EPS = 1e-5
NEG = -1000000000.0

_NT = (((1,), (1,)), ((), ()))


def _dot(a, b):
    return jnp.dot(a, b, preferred_element_type=F32)


def _dot_nt(a, b):
    return lax.dot_general(a, b, _NT, preferred_element_type=F32)


def _layernorm(x):
    m = jnp.mean(x, axis=-1, keepdims=True)
    xc = x - m
    v = jnp.mean(xc * xc, axis=-1, keepdims=True)
    return xc * lax.rsqrt(v + EPS)


def _ext(v):
    return jnp.concatenate([v, v[:, DM:D]], axis=1)


def _pair_block(y8, lo_mask):
    t = y8[:, DM:DE]
    zero = jnp.zeros_like(t)
    top = jnp.concatenate([y8[:, 0:DM], jnp.where(lo_mask, t, zero)], axis=1)
    bot = jnp.concatenate([y8[:, DE:PW], jnp.where(lo_mask, zero, t)], axis=1)
    return jnp.concatenate([top, bot], axis=0).astype(BF16)


def _group_allreduce(x, op, lane):
    for d in (1, 2, 4):
        up = pltpu.roll(x, d, 1)
        dn = pltpu.roll(x, 128 - d, 1)
        x = op(x, jnp.where((lane & d) != 0, up, dn))
    return x


def _kernel(x_hbm, mem0_ref, wq_hbm, wk_hbm, wv_hbm, wo_hbm, wr_ref, wg_hbm, wu_hbm,
            wd_hbm, c_ref, wmod_hbm, out_ref,
            x_v, wq_v, wk_v, wv_v, wo_v, wg_v, wu_v, wd_v, wmod_v,
            stq, stk, stv, wall, hext, kb, cur, mod_v, mem_v, best_v, bidx_v, sems):
    copies = [
        pltpu.make_async_copy(wq_hbm, wq_v, sems.at[0]),
        pltpu.make_async_copy(wk_hbm, wk_v, sems.at[1]),
        pltpu.make_async_copy(wv_hbm, wv_v, sems.at[2]),
        pltpu.make_async_copy(wo_hbm, wo_v, sems.at[3]),
        pltpu.make_async_copy(wmod_hbm, wmod_v, sems.at[4]),
        pltpu.make_async_copy(x_hbm, x_v, sems.at[5]),
        pltpu.make_async_copy(wg_hbm, wg_v, sems.at[6]),
        pltpu.make_async_copy(wu_hbm, wu_v, sems.at[7]),
        pltpu.make_async_copy(wd_hbm, wd_v, sems.at[8]),
    ]
    for cp in copies:
        cp.start()

    lane8 = lax.broadcasted_iota(jnp.int32, (8, 128), 1)
    lo_mask = lane8 < 64

    def stage(src, dst):
        def body(j, c):
            r = pl.multiple_of(j * 512, 512)
            r2 = pl.multiple_of(j * 256, 256)
            v = pltpu.bitcast(src[pl.ds(r, 512), :], jnp.uint32)
            dst[0, pl.ds(r2, 256), :] = v[:, :128]
            dst[1, pl.ds(r2, 256), :] = v[:, 128:]
            return c
        lax.fori_loop(0, (D * H) // 512, body, 0)

    def head_pair(st, p):
        u = jnp.concatenate(
            [st[0, pl.ds(p, D, stride=8), :], st[1, pl.ds(p, D, stride=8), :]], axis=1)
        lo = pltpu.bitcast(u << 16, F32).astype(BF16)
        hi = pltpu.bitcast(u & jnp.uint32(0xFFFF0000), F32).astype(BF16)
        return lo, hi

    copies[0].wait()
    stage(wq_v, stq)
    copies[1].wait()
    stage(wk_v, stk)

    scale = DH ** (-0.5)
    z64 = jnp.zeros((64, DH), BF16)
    for p in range(8):
        wq_e, wq_o = head_pair(stq, p)
        wk_e, wk_o = head_pair(stk, p)
        c, base = p // 2, (p % 2) * PW
        wall[c, :, base:base + DM] = (_dot_nt(wk_e, wq_e[0:DM]) * scale).astype(BF16)
        t = (_dot_nt(wk_e, jnp.concatenate([wq_e[DM:D], z64], axis=0))
             + _dot_nt(wk_o, jnp.concatenate([z64, wq_o[DM:D]], axis=0)))
        wall[c, :, base + DM:base + DE] = (t * scale).astype(BF16)
        wall[c, :, base + DE:base + PW] = (_dot_nt(wk_o, wq_o[0:DM]) * scale).astype(BF16)

    copies[2].wait()
    stage(wv_v, stv)
    copies[3].wait()
    zc = jnp.zeros((DH, 64), BF16)
    for p in range(8):
        wv_e, wv_o = head_pair(stv, p)
        wo_e = wo_v[(2 * p) * DH:(2 * p + 1) * DH, :]
        wo_o = wo_v[(2 * p + 1) * DH:(2 * p + 2) * DH, :]
        c, base = 4 + p // 2, (p % 2) * PW
        wall[c, :, base:base + DM] = _dot(wv_e, wo_e[:, 0:DM]).astype(BF16)
        t = (_dot(wv_e, jnp.concatenate([wo_e[:, DM:D], zc], axis=1))
             + _dot(wv_o, jnp.concatenate([zc, wo_o[:, DM:D]], axis=1)))
        wall[c, :, base + DM:base + DE] = t.astype(BF16)
        wall[c, :, base + DE:base + PW] = _dot(wv_o, wo_o[:, 0:DM]).astype(BF16)

    copies[4].wait()
    cf = c_ref[...].astype(F32)
    sc = (cf * jax.nn.sigmoid(cf)).astype(BF16)
    mod = _dot(jnp.broadcast_to(sc, (8, D)), wmod_v[...])
    for k in range(6):
        mod_v[k] = mod[:, k * D:(k + 1) * D]

    copies[5].wait()

    def ln1(b, c):
        r = pl.multiple_of(b * 128, 128)
        xf = x_v[pl.ds(r, 128), :].astype(F32)
        h = _layernorm(xf) * (1.0 + mod_v[1][0:1]) + mod_v[0][0:1]
        hext[pl.ds(b * 4, 4)] = _ext(h).reshape(4, SEG, DE)
        return c
    lax.fori_loop(0, S // 128, ln1, 0)

    def bulk(b, c):
        lhs = hext[pl.ds(b * 16, 16), 0:8, :].reshape(128, DE)[:, 0:D].astype(BF16)
        for ch in range(NCH):
            for pp in range(2):
                y = _dot(lhs, wall[ch, :, pp * PW:(pp + 1) * PW])
                prow = ((ch % 4) * 2 + pp) * 16
                for r in range(16):
                    kb[b * 16 + r, ch // 4, prow:prow + 16, :] = _pair_block(
                        y[r * 8:(r + 1) * 8], lo_mask)
        return c
    lax.fori_loop(0, NSEG // 16, bulk, 0)

    mem_v[...] = _ext(mem0_ref[...].astype(F32))
    best_v[...] = jnp.full(best_v.shape, -jnp.inf, F32)
    bidx_v[...] = jnp.zeros(bidx_v.shape, jnp.int32)

    row8 = lax.broadcasted_iota(jnp.int32, (8, 128), 0)
    tri = row8 >= (lane8 & 7)
    qkey = (0, 4, 3, 2, 1)
    cur_of_key = {0: 0, 4: 1, 3: 2, 2: 3}

    def step(s, carry):
        hs = hext[s]
        q = jnp.concatenate([mem_v[...], hs[24:32], hs[16:24], hs[8:16], hs[0:8]], axis=0)
        qb = q.astype(BF16)
        lhs = qb[0:32, 0:D]
        for ch in range(NCH):
            for pp in range(2):
                y = _dot(lhs, wall[ch, :, pp * PW:(pp + 1) * PW])
                prow = ((ch % 4) * 2 + pp) * 16
                for r in range(4):
                    cur[ch // 4, r, prow:prow + 16, :] = _pair_block(
                        y[r * 8:(r + 1) * 8], lo_mask)

        def stack(gu, g):
            return kb[s, gu] if g == 1 else cur[gu, cur_of_key[g]]

        sc_g = [_dot_nt(qb, stack(0, g)) for g in range(5)]
        p_rows = []
        for qi in range(5):
            vis = range(5) if qi == 0 else range(qkey[qi] + 1)
            vals = {}
            for g in vis:
                v = sc_g[g][qi * 8:(qi + 1) * 8]
                if qi != 0 and g == qkey[qi]:
                    v = jnp.where(tri, v, NEG)
                vals[g] = v
            mx = functools.reduce(jnp.maximum, vals.values())
            mx = _group_allreduce(mx, jnp.maximum, lane8)
            ex = {g: jnp.exp(v - mx) for g, v in vals.items()}
            sm = functools.reduce(jnp.add, ex.values())
            sm = _group_allreduce(sm, jnp.add, lane8)
            inv = 1.0 / sm
            p_rows.append([ex[g] * inv if g in ex else jnp.zeros((8, 128), F32)
                           for g in range(5)])
        o = None
        for g in range(5):
            pg = jnp.concatenate([p_rows[qi][g] for qi in range(5)], axis=0).astype(BF16)
            og = _dot(pg, stack(1, g))
            o = og if o is None else o + og
        ot = o[:, DM:DE]
        ot = ot + pltpu.roll(ot, 64, 1)
        oext = jnp.concatenate([o[:, 0:DM], ot], axis=1)
        mem_v[...] = oext[0:8]

        attn = jnp.concatenate([oext[32:40], oext[24:32], oext[16:24], oext[8:16]],
                               axis=0)[:, 0:D]
        r0 = pl.multiple_of(s * SEG, SEG)
        x2 = x_v[pl.ds(r0, SEG), :].astype(F32) + mod_v[2][0:1] * attn
        h2 = _layernorm(x2) * (1.0 + mod_v[4][0:1]) + mod_v[3][0:1]
        out_ref[pl.ds(r0, SEG), :] = (x2 + mod_v[5][0:1] * h2).astype(BF16)
        hext[s, :, 0:D] = h2
        rr = jnp.sum(h2 * wr_ref[...].astype(F32), axis=-1, keepdims=True)
        rb = jnp.broadcast_to(rr, (SEG, 128))
        better = rb > best_v[...]
        best_v[...] = jnp.where(better, rb, best_v[...])
        bidx_v[...] = jnp.where(better, s, bidx_v[...])
        return carry
    lax.fori_loop(0, NSEG, step, 0)

    best = best_v[...]
    rmax = jnp.max(best)
    tok = bidx_v[...] * SEG + lax.broadcasted_iota(jnp.int32, (SEG, 128), 0)
    idx = jnp.min(jnp.where(best == rmax, tok, S - 1))
    idx = jnp.clip(idx, 0, S - 1)
    sidx = idx // SEG
    ridx = idx % SEG
    hseg = hext[sidx][:, 0:D]
    rows = lax.broadcasted_iota(jnp.int32, (SEG, D), 0)
    xsel = jnp.sum(jnp.where(rows == ridx, hseg, 0.0), axis=0, keepdims=True)
    xsel = jnp.broadcast_to(xsel, (8, D)).astype(BF16)
    copies[6].wait()
    copies[7].wait()
    copies[8].wait()
    gt = _dot(xsel, wg_v[...])
    gt = gt * jax.nn.sigmoid(gt)
    up = _dot(xsel, wu_v[...])
    y = _dot((gt * up).astype(BF16), wd_v[...])
    rsel = jax.nn.sigmoid(jnp.max(best, axis=0, keepdims=True)[:, 0:1])
    upd = mod_v[5][0:1] * (y[0:1] * rsel)
    r0 = pl.multiple_of(sidx * SEG, SEG)
    blk = out_ref[pl.ds(r0, SEG), :].astype(F32)
    out_ref[pl.ds(r0, SEG), :] = jnp.where(rows == ridx, blk + upd, blk).astype(BF16)


def pallas_adaLN_cond__memory_aug_recurrent_mem_tr__moe_arch_mod__prompt_kernel(
    A_x, A_mem0, A_Wq, A_Wk, A_Wv, A_Wo, A_seg_len, B_x, B_w_r, B_w_gate, B_w_up,
    B_w_down, c, w_mod,
):
    assert isinstance(A_seg_len, int) and A_seg_len == SEG
    assert A_x.shape == (1, S, D) and A_Wq.shape == (D, H, DH) and A_mem0.shape == (1, M, D)
    del B_x
    any_spec = pl.BlockSpec(memory_space=pl.ANY)
    vmem_spec = pl.BlockSpec(memory_space=pltpu.VMEM)
    out = pl.pallas_call(
        _kernel,
        out_shape=jax.ShapeDtypeStruct((S, D), BF16),
        in_specs=[any_spec, vmem_spec, any_spec, any_spec, any_spec, any_spec, vmem_spec,
                  any_spec, any_spec, any_spec, vmem_spec, any_spec],
        out_specs=vmem_spec,
        scratch_shapes=[
            pltpu.VMEM((S, D), BF16),
            pltpu.VMEM((D * H, DH), BF16),
            pltpu.VMEM((D * H, DH), BF16),
            pltpu.VMEM((D * H, DH), BF16),
            pltpu.VMEM((H * DH, D), BF16),
            pltpu.VMEM((D, FF), BF16),
            pltpu.VMEM((D, FF), BF16),
            pltpu.VMEM((FF, D), BF16),
            pltpu.VMEM((D, 6 * D), BF16),
            pltpu.VMEM((2, D * H // 2, 128), jnp.uint32),
            pltpu.VMEM((2, D * H // 2, 128), jnp.uint32),
            pltpu.VMEM((2, D * H // 2, 128), jnp.uint32),
            pltpu.VMEM((NCH, D, CW), BF16),
            pltpu.VMEM((NSEG, SEG, DE), F32),
            pltpu.VMEM((NSEG, 2, 128, DE), BF16),
            pltpu.VMEM((2, 4, 128, DE), BF16),
            pltpu.VMEM((6, 8, D), F32),
            pltpu.VMEM((M, DE), F32),
            pltpu.VMEM((SEG, 128), F32),
            pltpu.VMEM((SEG, 128), jnp.int32),
            pltpu.SemaphoreType.DMA((9,)),
        ],
        compiler_params=pltpu.CompilerParams(vmem_limit_bytes=120 * 1024 * 1024),
    )(
        A_x.reshape(S, D), A_mem0.reshape(M, D),
        A_Wq.reshape(D * H, DH), A_Wk.reshape(D * H, DH), A_Wv.reshape(D * H, DH),
        A_Wo.reshape(H * DH, D), B_w_r.reshape(1, D), B_w_gate, B_w_up, B_w_down,
        c, w_mod,
    )
    return out.reshape(1, S, D)
```

```python
import functools

import jax
import jax.numpy as jnp
from jax import lax
import jax.experimental.pallas as pl
import jax.experimental.pallas.tpu as pltpu

F32 = jnp.float32
BF16 = jnp.bfloat16

S = 2048
D = 448
H = 16
DH = 256
M = 8
SEG = 32
NSEG = S // SEG
FF = 1792
DM = 384
DE = 512
NP = H // 2
TPP = 7
NT = 2 * NP * TPP
BSEG = 8
NBLK = S // 128
UNROLL1 = 4
UNROLL2 = 2
CHUNKS = ((0, 128), (128, 128), (256, 128), (384, 64))
XA = 2 * BSEG * SEG
WAIT_GROUPS = (
    ("q00",),
    ("k00",),
    ("q01",),
    ("k01",),
    ("q02",),
    ("k02", "q03"),
    ("k03", "q10", "k10"),
    ("q11", "k11"),
    ("q12", "k12"),
    ("q13", "k13", "c", "m0", "wr", "ma", "xa"),
    ("v0", "o0"),
    ("o1",),
    ("xc", "v1", "o2"),
    ("o3", "mb"),
    ("xb",),
    ("wg", "wu", "wd"),
)
NTAIL = 10
EPS = 1e-5
NEG = -1000000000.0

_NT = (((1,), (1,)), ((), ()))


def _dot(a, b):
    return jnp.dot(a, b, preferred_element_type=F32)


def _dot_nt(a, b):
    return lax.dot_general(a, b, _NT, preferred_element_type=F32)


def _as_words(x):
    return pltpu.bitcast(x, jnp.uint32)


def _as_bf16(x):
    return pltpu.bitcast(x, BF16)


def _cat(xs, axis):
    return jnp.concatenate(xs, axis=axis)


def _group_allreduce(x, op, lane):
    for d in (1, 2, 4):
        up = pltpu.roll(x, d, 1)
        dn = pltpu.roll(x, 128 - d, 1)
        x = op(x, jnp.where((lane & d) != 0, up, dn))
    return x


def _ln_tiles(t, lo, w=None):
    t3 = jnp.where(lo, t[3], 0.0)
    m = jnp.sum(t[0] + t[1] + t[2] + t3, axis=-1, keepdims=True) * (1.0 / D)
    c = [ti - m for ti in t]
    c3 = jnp.where(lo, c[3], 0.0)
    v = jnp.sum(c[0] * c[0] + c[1] * c[1] + c[2] * c[2] + c3 * c3,
                axis=-1, keepdims=True) * (1.0 / D)
    rs = lax.rsqrt(v + EPS)
    n = [ci * rs for ci in c]
    if w is None:
        return n
    d = jnp.sum(c[0] * w[0] + c[1] * w[1] + c[2] * w[2] + c[3] * w[3], axis=-1, keepdims=True)
    return n, d * rs


def _kernel(xt_hbm, mem0_hbm, wq_hbm, wk_hbm, wv_hbm, wot_hbm, wr_hbm, wg_hbm, wu_hbm,
            wdt_hbm, c_hbm, wmod_hbm, out_hbm,
            xt_v, wq_v, wk_v, wv_v, wot_v, wg_v, wu_v, wdt_v, wmod_v,
            stq, stk, stv, wall, wb, hp, xr, orow, besth, kb, kq, cur, oprev, outt,
            mod_v, best_v, bidx_v, mem0_ref, wr_ref, c_ref, sems):
    cps = {}

    def add_copy(name, src, dst):
        (sem,) = [i for i, g in enumerate(WAIT_GROUPS) if name in g]
        cps[name] = pltpu.make_async_copy(src, dst, sems.at[sem])

    def add_v(hh):
        add_copy("v" + str(hh), wv_hbm.at[:, pl.ds(8 * hh, 8), :], wv_v.at[hh])

    def add_o(j):
        add_copy("o" + str(j), wot_hbm.at[pl.ds(4 * j, 4)], wot_v.at[pl.ds(4 * j, 4)])

    def add_half(name, hbm, vm, hh, i):
        d0, n = CHUNKS[i]
        add_copy(name + str(hh) + str(i), hbm.at[pl.ds(d0, n), pl.ds(8 * hh, 8), :],
                 vm.at[hh, pl.ds(d0, n)])

    for hh in range(2):
        for i in range(4):
            add_half("q", wq_hbm, wq_v, hh, i)
            add_half("k", wk_hbm, wk_v, hh, i)
    add_copy("c", c_hbm, c_ref)
    add_copy("m0", mem0_hbm, mem0_ref)
    add_copy("wr", wr_hbm, wr_ref)
    add_copy("ma", wmod_hbm.at[:, pl.ds(0, 2 * D)], wmod_v.at[:, pl.ds(0, 2 * D)])
    add_copy("xa", xt_hbm.at[:, pl.ds(0, XA // 2)], xt_v.at[:, pl.ds(0, XA // 2)])
    add_v(0)
    add_o(0)
    add_o(1)
    add_copy("xc", xt_hbm.at[:, pl.ds(XA // 2, XA // 2)], xt_v.at[:, pl.ds(XA // 2, XA // 2)])
    add_v(1)
    add_o(2)
    add_o(3)
    add_copy("mb", wmod_hbm.at[:, pl.ds(2 * D, 4 * D)], wmod_v.at[:, pl.ds(2 * D, 4 * D)])
    add_copy("xb", xt_hbm.at[:, pl.ds(XA, S - XA)], xt_v.at[:, pl.ds(XA, S - XA)])
    add_copy("wg", wg_hbm, wg_v)
    add_copy("wu", wu_hbm, wu_v)
    add_copy("wd", wdt_hbm, wdt_v)
    assert len(cps) == sum(len(g) for g in WAIT_GROUPS)
    late = ("wg", "wu", "wd")
    for nm, cp in cps.items():
        if nm not in late:
            cp.start()

    def out_copy(b, sem=0):
        return pltpu.make_async_copy(
            outt.at[b, pl.ds(0, D), :],
            out_hbm.at[:, pl.ds(pl.multiple_of(b * 128, 128), 128)],
            sems.at[sem])

    lane8 = lax.broadcasted_iota(jnp.int32, (8, 128), 1)

    def lo_mask(rows):
        return lax.broadcasted_iota(jnp.int32, (rows, 128), 1) < 64

    def stage_half(src, st, hh, i):
        d0, n = CHUNKS[i]
        for sub in range(d0, d0 + n, 32):
            v = pltpu.bitcast(src[hh, sub:sub + 32].reshape(256, DH), jnp.uint32)
            st[hh, 0, sub * 4:(sub + 32) * 4, :] = v[:, :128]
            st[hh, 1, sub * 4:(sub + 32) * 4, :] = v[:, 128:]

    def pair_rows_half(st, p, r0, r1):
        u = _cat([st[p // 4, c, pl.ds(r0 * 4 + p % 4, r1 - r0, stride=4), :] for c in range(2)], 1)
        return (pltpu.bitcast(u << 16, F32).astype(BF16),
                pltpu.bitcast(u & jnp.uint32(0xFFFF0000), F32).astype(BF16))

    z64 = jnp.zeros((64, DH), BF16)

    def fuse(gu, p, r0, r1, tiles, lhs, rhs, scale):
        base = (gu * NP + p) * TPP

        def put(idx, y):
            if scale is not None:
                y = y * scale
            wall[idx, r0 // 2:r1 // 2, :] = _as_words(y.astype(BF16))

        l_e, l_o = lhs(p, r0, r1)
        for t in sorted(tiles, reverse=True):
            if t < 3:
                r_e, r_o = rhs(p, t * 128, (t + 1) * 128)
                put(base + t, _dot_nt(l_e, r_e))
                put(base + 4 + t, _dot_nt(l_o, r_o))
            else:
                r_e, r_o = rhs(p, DM, D)
                for a in range(0, r1 - r0, 128):
                    n = min(128, r1 - r0 - a)
                    s_e, s_o = l_e[a:a + n], l_o[a:a + n]
                    if n < 128:
                        s_e, s_o = _cat([s_e, z64], 0), _cat([s_o, z64], 0)
                    y = _cat([_dot_nt(r_e, s_e), _dot_nt(r_o, s_o)], 0)
                    if scale is not None:
                        y = y * scale
                    wall[base + 3, (r0 + a) // 2:(r0 + a + n) // 2, :] = _as_words(y.T[0:n].astype(BF16))

    def fuse_a(hh, r0, r1, tiles):
        return [functools.partial(fuse, 0, p, r0, r1, tiles,
                                  functools.partial(pair_rows_half, stk),
                                  functools.partial(pair_rows_half, stq), DH ** (-0.5))
                for p in range(4 * hh, 4 * hh + 4)]

    def fuse_q(hh):
        def one(p):
            l_e, l_o = pair_rows_half(stk, p, DM, D)
            for t in range(4):
                n = 128 if t < 3 else 64
                r_e, r_o = pair_rows_half(stq, p, t * 128, t * 128 + n)
                if n < 128:
                    r_e, r_o = _cat([r_e, z64], 0), _cat([r_o, z64], 0)
                y = _cat([_dot_nt(l_e, r_e), _dot_nt(l_o, r_o)], 0) * DH ** (-0.5)
                wall[NT + p, t * 64:t * 64 + n // 2, :] = _as_words(y.T[0:n].astype(BF16))

        return [functools.partial(one, p) for p in range(4 * hh, 4 * hh + 4)]

    def fuse_b(r0, r1, groups):
        def rhs(p, a, b):
            return wot_v[2 * p, a:b, :], wot_v[2 * p + 1, a:b, :]

        return [functools.partial(fuse, 1, p, r0, r1, range(4), functools.partial(pair_rows_half, stv), rhs, None)
                for j in groups for p in (2 * j, 2 * j + 1)]

    def fuse_z(groups):
        def one(p):
            l_e, l_o = pair_rows_half(stv, p, DM, D)
            for t in range(4):
                n = 128 if t < 3 else 64
                r_e = wot_v[2 * p, t * 128:t * 128 + n, :]
                r_o = wot_v[2 * p + 1, t * 128:t * 128 + n, :]
                if n < 128:
                    r_e, r_o = _cat([r_e, z64], 0), _cat([r_o, z64], 0)
                wb[p, t] = _as_words(_cat([_dot_nt(l_e, r_e), _dot_nt(l_o, r_o)], 0).astype(BF16))

        return [functools.partial(one, p) for j in groups for p in (2 * j, 2 * j + 1)]

    def run(main, side=()):
        side = list(side)
        done = 0
        for i, th in enumerate(main):
            th()
            upto = (i + 1) * len(side) // len(main)
            for sd in side[done:upto]:
                sd()
            done = upto

    zpad = jnp.zeros((8, DE - D), F32)

    def mod_thunks(k0, k1):
        parts = []

        def tile(i):
            cf = c_ref[...].astype(F32)
            sc = (cf * jax.nn.sigmoid(cf)).astype(BF16)
            parts.append(_dot(jnp.broadcast_to(sc, (8, D)), wmod_v[:, i * 128:(i + 1) * 128]))

        def store():
            mod = _cat(parts, 1)
            for k in range(k0, k1):
                v = mod[:, (k - k0) * D:(k - k0 + 1) * D]
                if k in (1, 4):
                    v = v + 1.0
                mod_v[k] = _cat([v, v[:, DM:D]], 1)

        return [functools.partial(tile, i) for i in range(k0 * D // 128, k1 * D // 128)] + [store]

    def modt(k, j):
        return mod_v[k, 0:1, j * 128:(j + 1) * 128]

    def ln1(b):
        col = b * 128 if isinstance(b, int) else pl.multiple_of(b * 128, 128)
        xb = xt_v[:, pl.ds(col, 128)].astype(F32)
        xb = _cat([xb, xb[DM:D]], 0)
        t = [xb[j * 128:(j + 1) * 128].T for j in range(4)]
        n = _ln_tiles(t, lo_mask(128))
        for j in range(4):
            xr[j, pl.ds(b * 4, 4)] = t[j].reshape(4, SEG, 128)
            hp[j, pl.ds(b * 4, 4)] = (n[j] * modt(1, j) + modt(0, j)).reshape(4, SEG, 128)

    def pack2(a, b):
        return _as_words(_cat([a, b], 0).astype(BF16))

    def split(y):
        return _cat([jnp.where(lane8 < 64, y, 0.0), jnp.where(lane8 < 64, 0.0, y)], 0)

    def fold(y):
        return y + pltpu.roll(y, 64, 1)

    def xdot(lhs, idxs):
        return _dot(lhs[:, 0:DM], _cat([_as_bf16(wall[i, 0:DM // 2, :]) for i in idxs], 1))

    def bulk_lhs(bb):
        return _cat([hp[j, pl.ds(bb * BSEG, BSEG), 0:8, :].reshape(BSEG * 8, 128)
                     for j in range(4)], 1)[:, 0:D].astype(BF16)

    def bulk_thunks(lhs, bb, gu, p):
        base = (gu * NP + p) * TPP
        held = {}

        def tail(y):
            for r in range(BSEG):
                kb[bb * BSEG + r, gu, p, 3] = _as_words(split(y[r * 8:(r + 1) * 8]).astype(BF16))

        def even(t, y):
            held[t] = y

        def odd(t, y):
            for r in range(BSEG):
                kb[bb * BSEG + r, gu, p, t] = pack2(held[t][r * 8:(r + 1) * 8],
                                                    y[r * 8:(r + 1) * 8])

        def qside(y):
            kq[pl.ds(bb * BSEG, BSEG), p] = y.reshape(BSEG, 8, 128)

        def ktiles(idx, kdim, finish):
            parts = []

            def one(k0):
                k1 = min(k0 + 128, kdim)
                parts.append(_dot(lhs[:, k0:k1], _as_bf16(wall[idx, k0 // 2:k1 // 2, :])))
                if k1 == kdim:
                    finish(functools.reduce(jnp.add, parts))

            return [functools.partial(one, k0) for k0 in range(0, kdim, 128)]

        out = ktiles(NT + p, D, qside) if gu == 0 else []
        out += ktiles(base + 3, DM, tail)
        for t in range(3):
            out += ktiles(base + t, DM, functools.partial(even, t))
            out += ktiles(base + 4 + t, DM, functools.partial(odd, t))
        return out

    def wait(*names):
        assert names in WAIT_GROUPS
        for nm in names:
            cps[nm].wait()

    def prepass(gu):
        lhs = bulk_lhs(0)
        return [th for p in range(NP) for th in bulk_thunks(lhs, 0, gu, p)]

    def ln1s(b0, b1):
        return [functools.partial(ln1, b) for b in range(b0, b1)]

    best_v[...] = jnp.full(best_v.shape, -jnp.inf, F32)
    bidx_v[...] = jnp.zeros(bidx_v.shape, jnp.int32)
    oprev[...] = jnp.zeros(oprev.shape, F32)
    besth[...] = jnp.zeros(besth.shape, F32)
    orow[:, 0:4] = jnp.zeros((4, 4, SEG, 128), F32)

    nb0 = XA // 128
    wait("q00")
    stage_half(wq_v, stq, 0, 0)
    wait("k00")
    stage_half(wk_v, stk, 0, 0)
    run(fuse_a(0, 0, 128, (0,)))
    wait("q01")
    stage_half(wq_v, stq, 0, 1)
    run(fuse_a(0, 0, 128, (1,)))
    wait("k01")
    stage_half(wk_v, stk, 0, 1)
    run(fuse_a(0, 128, 256, (0, 1)))
    wait("q02")
    stage_half(wq_v, stq, 0, 2)
    run(fuse_a(0, 0, 256, (2,)))
    wait("k02", "q03")
    stage_half(wk_v, stk, 0, 2)
    stage_half(wq_v, stq, 0, 3)
    run(fuse_a(0, 0, 256, (3,)) + fuse_a(0, 256, 384, (0, 1, 2, 3)))
    wait("k03", "q10", "k10")
    stage_half(wk_v, stk, 0, 3)
    stage_half(wq_v, stq, 1, 0)
    stage_half(wk_v, stk, 1, 0)
    run(fuse_q(0) + fuse_a(1, 0, 128, (0,)))
    wait("q11", "k11")
    stage_half(wq_v, stq, 1, 1)
    stage_half(wk_v, stk, 1, 1)
    run(fuse_a(1, 128, 256, (0,)) + fuse_a(1, 0, 256, (1,)))
    wait("q12", "k12")
    stage_half(wq_v, stq, 1, 2)
    stage_half(wk_v, stk, 1, 2)
    run(fuse_a(1, 256, 384, (0, 1)) + fuse_a(1, 0, 384, (2,)))
    wait("q13", "k13", "c", "m0", "wr", "ma", "xa")
    run(mod_thunks(0, 2))
    stage_half(wq_v, stq, 1, 3)
    stage_half(wk_v, stk, 1, 3)
    run(fuse_a(1, 0, 384, (3,)) + fuse_q(1), ln1s(0, 2))
    run(prepass(0)[:175])
    wait("v0", "o0")
    run(prepass(0)[175:])
    for i in range(4):
        stage_half(wv_v, stv, 0, i)
    run(fuse_b(0, 128, (0,)) + fuse_b(128, 256, (0,)) + fuse_b(256, DM, (0,)) + fuse_z((0,)))
    wait("o1")
    run(fuse_z((1,)) + fuse_b(0, DM, (1,)))
    wait("xc", "v1", "o2")
    pu = prepass(1)
    run(pu[:42])
    for i in range(4):
        stage_half(wv_v, stv, 1, i)
    run(fuse_b(0, 128, (2,)) + fuse_b(128, 256, (2,)) + fuse_b(256, DM, (2,)) + fuse_z((2,)) + pu[42:84],
        ln1s(2, nb0))
    wait("o3", "mb")
    m0 = mem0_ref[...].astype(F32)
    m0 = _cat([m0, m0[:, DM:D]], 1)
    mem = [m0[:, j * 128:(j + 1) * 128] for j in range(4)]
    pu = prepass(1)
    run(fuse_z((3,)) + fuse_b(0, DM, (3,)))
    run(pu[84:144], mod_thunks(2, 6))
    wr = _cat([jnp.broadcast_to(wr_ref[...].astype(F32).reshape(1, D), (8, D)), zpad], 1)
    mod_v[6] = mod_v[4] * wr
    mod_v[7] = jnp.broadcast_to(
        jnp.sum(mod_v[3] * wr, axis=-1, keepdims=True), (8, DE))
    run(pu[144:])
    wait("xb")

    for nm in late:
        cps[nm].start()

    row8 = lax.broadcasted_iota(jnp.int32, (8, 128), 0)
    tri = row8 >= (lane8 & 7)
    qkey = (0, 4, 3, 2, 1)
    cur_of_key = {0: 0, 4: 1, 3: 2, 2: 3}
    qrows = (40, 40, 32, 32, 16)

    def epilogue(sp, valid, slot):
        lo = lo_mask(SEG)
        attn = [oprev[slot, 0], oprev[slot, 1], oprev[slot, 2], fold(oprev[slot, 3])]
        x2 = [xr[j, sp] + modt(2, j) * attn[j] for j in range(4)]
        n, nw = _ln_tiles(x2, lo, [modt(6, j) for j in range(4)])
        h2 = [n[j] * modt(4, j) + modt(3, j) for j in range(4)]
        for j in range(4):
            orow[j, sp] = x2[j] + modt(5, j) * h2[j]
        rb = nw + modt(7, 0)
        better = rb > best_v[...]
        if valid is not None:
            better = jnp.logical_and(better, valid)
        best_v[...] = jnp.where(better, rb, best_v[...])
        bidx_v[...] = jnp.where(better, sp, bidx_v[...])
        for j in range(4):
            besth[j] = jnp.where(better, h2[j], besth[j])

    def transpose_out(b, j):
        blk = orow[j, pl.ds(b * 4, 4)].reshape(128, 128)
        row = j * 128 if isinstance(j, int) else pl.multiple_of(j * 128, 128)
        outt[b, pl.ds(row, 128), :] = blk.T.astype(BF16)

    def main_tails(lhs, gu):
        for pp in range(NP // 2):
            b0 = (gu * NP + 2 * pp) * TPP + 3
            y = xdot(lhs, [b0, b0 + TPP])
            for i in range(2):
                yt = y[:, i * 128:(i + 1) * 128]
                for r in range(4):
                    cur[gu, r, 3, 2 * pp + i] = _as_words(split(yt[r * 8:(r + 1) * 8]).astype(BF16))

    def main_tile(lhs, gu, t):
        for p in range(NP):
            base = (gu * NP + p) * TPP
            y = xdot(lhs, [base + t, base + 4 + t])
            for r in range(4):
                cur[gu, r, t, p] = pack2(y[r * 8:(r + 1) * 8, 0:128], y[r * 8:(r + 1) * 8, 128:256])

    def step(s, mem, with_bulk, deferred, last, par, held):
        hs = [hp[j, s] for j in range(4)]
        qb = _cat([_cat([mem[j], hs[j][24:32], hs[j][16:24], hs[j][8:16], hs[j][0:8]], 0)
                   for j in range(4)], 1).astype(BF16)
        lhs = qb[0:32, 0:D]

        def stack(gu, g, t):
            v = kb[s, gu, :, t] if g == 1 else cur[gu, cur_of_key[g], t]
            return _as_bf16(v.reshape(64, 128))

        hb = [mem[3]] + [hs[3][8 * k:8 * k + 8] for k in range(4)]
        tb = [split(v) for v in hb] + [jnp.zeros((16, 128), F32)] * 3
        tt = _cat(tb, 0).astype(BF16)
        qs = [_dot(lhs, _cat([_as_bf16(wall[NT + p]), _as_bf16(wall[NT + p + 1])], 1))
              for p in range(0, NP, 2)]
        main_tails(lhs, 0)
        rot = {}
        for i, y in enumerate(qs):
            p = 2 * i
            ql = _cat([y[:, 0:128], y[:, 128:256], kq[s, p], kq[s, p + 1]], 0).astype(BF16)
            r = _dot_nt(ql, tt)
            for k in range(2):
                rk = _cat([r[32 * k:32 * k + 32], r[64 + 8 * k:72 + 8 * k]], 0)
                rot[p + k] = pltpu.roll(rk, 16 * (p + k), 1) if p + k else rk

        def s2(qi, g):
            rows = slice(qi * 8, (qi + 1) * 8)
            c = rot[0][rows]
            for p in range(1, NP):
                c = jnp.where((lane8 >> 4) == (p + g) % NP, rot[p][rows], c)
            return pltpu.roll(c, 128 - 16 * g, 1) if g else c

        for t in range(3):
            main_tile(lhs, 0, t)
        main_tails(lhs, 1)

        fill = []
        if with_bulk:
            bb = s // BSEG + 1
            blhs = bulk_lhs(bb)
            fg = bulk_thunks(blhs, bb, 0, s % BSEG)
            fu = bulk_thunks(blhs, bb, 1, s % BSEG)
            fill = fg[:7] + fu[:3] + fg[7:] + fu[3:]

        def emit(n):
            for th in fill[:n]:
                th()
            del fill[:n]

        sc_g = {}
        for g in (1, 2, 3, 4, 0):
            emit(4)
            sc_g[g] = _dot_nt(qb[0:qrows[g]], _cat([stack(0, g, t) for t in range(4)], 1))

        for t in range(3):
            main_tile(lhs, 1, t)

        epilogue(jnp.maximum(s - 2, 0), s > 1, par)
        tq = jnp.maximum(s - 6, 0)
        transpose_out(tq // 4, tq % 4)

        p_rows = []
        d_rows = [[] for _ in range(NP)]
        for qi in range(5):
            vis = range(5) if qi == 0 else range(qkey[qi] + 1)
            vals = {}
            for g in vis:
                v = sc_g[g][qi * 8:(qi + 1) * 8] + s2(qi, g)
                if qi != 0 and g == qkey[qi]:
                    v = jnp.where(tri, v, NEG)
                vals[g] = v
            mx = functools.reduce(jnp.maximum, vals.values())
            mx = _group_allreduce(mx, jnp.maximum, lane8)
            ex = {g: jnp.exp(v - mx) for g, v in vals.items()}
            sm = functools.reduce(jnp.add, ex.values())
            sm = _group_allreduce(sm, jnp.add, lane8)
            inv = 1.0 / sm
            pn = {g: e * inv for g, e in ex.items()}
            p_rows.append(_cat([pn[g] if g in pn else jnp.zeros((8, 128), F32)
                                for g in range(5)], 1))
            pr = {g: pltpu.roll(v, 16 * g, 1) if g else v for g, v in pn.items()}
            for p in range(NP):
                d = jnp.zeros((8, 128), F32)
                for g, v in pr.items():
                    d = jnp.where((lane8 >> 4) == (p + g) % NP, v, d)
                d_rows[p].append(d)
        pall = _cat(p_rows, 0).astype(BF16)
        zs = [_dot(_cat(d_rows[p], 0).astype(BF16),
                   _cat([tb[(b - p) % NP] for b in range(NP)], 0).astype(BF16))
              for p in range(NP)]
        o = {}
        o1 = _dot(pall[:, 128:256], _cat([stack(1, 1, t) for t in range(4)], 1))
        for t in (0, 1, 3, 2):
            oa = _dot(pall[:, 0:128], stack(1, 0, t)) + o1[:, t * 128:(t + 1) * 128]
            oc = _dot(pall[0:16, 512:640], stack(1, 4, t))
            ob = _dot(pall[0:32, 256:512], _cat([stack(1, g, t) for g in (2, 3)], 0))
            o[t] = oa[0:32] + ob
            o[t] = _cat([o[t][0:16] + oc, o[t][16:32], oa[32:40]], 0)
        zc = _cat(zs, 1)
        if par == 0:
            held["z"], held["o"] = zc[32:40], [o[t][32:40] for t in range(4)]
            zc = zc[0:32]
        else:
            zc = _cat([zc, held["z"]], 0)
        zc = zc.astype(BF16)
        for t in (3, 0, 1, 2):
            oz = _dot(zc, _as_bf16(wb[:, t].reshape(NP * 64, 128)))
            ot = o[t]
            o[t] = ot[0:32] + oz[0:32]
            oprev[par, t, 8:32] = _cat([o[t][24:32], o[t][16:24], o[t][8:16]], 0)
            if par == 1:
                oprev[1, t, 0:8] = ot[32:40] + oz[32:40]
                oprev[0, t, 0:8] = held["o"][t] + oz[40:48]
        mem_next = [o[0][0:8], o[1][0:8], o[2][0:8], fold(o[3][0:8])]

        if not last:
            deferred += fill[NTAIL:]
            fill = fill[:NTAIL]
        else:
            fill = fill + deferred
        for th in fill:
            th()
        return mem_next

    def steps(i, mem, with_bulk, unroll):
        deferred, held = [], {}
        for u in range(unroll):
            mem = step(i * unroll + u, mem, with_bulk, deferred, u == unroll - 1, u % 2, held)
        if with_bulk:
            assert unroll == 4
            ln1(jnp.minimum(i + nb0, NBLK - 1))
        for u in range(0, unroll, 4):
            s = i * unroll + u

            @pl.when(jnp.logical_and(s >= 8, s % 4 == 0))
            def _():
                out_copy(s // 4 - 2).start()
        return mem

    n1 = NSEG - BSEG
    mem = lax.fori_loop(0, n1 // UNROLL1,
                        functools.partial(steps, with_bulk=True, unroll=UNROLL1), mem)
    wait(*late)
    mem = lax.fori_loop(n1 // UNROLL2, NSEG // UNROLL2,
                        functools.partial(steps, with_bulk=False, unroll=UNROLL2), mem)

    epilogue(NSEG - 2, None, 0)
    epilogue(NSEG - 1, None, 1)
    transpose_out(NBLK - 2, 2)
    transpose_out(NBLK - 2, 3)
    out_copy(NBLK - 2, 1).start()
    for j in range(4):
        transpose_out(NBLK - 1, j)
    out_copy(NBLK - 1, 1).start()

    best = best_v[...]
    rmax = jnp.max(best, axis=0, keepdims=True)
    tok = bidx_v[...] * SEG + lax.broadcasted_iota(jnp.int32, (SEG, 128), 0)
    tmin = jnp.min(jnp.where(best == rmax, tok, S - 1), axis=0, keepdims=True)
    sel = tok == tmin
    xsel = _cat([jnp.sum(jnp.where(sel, besth[j], 0.0), axis=0, keepdims=True)
                 for j in range(4)], 1)[:, 0:D]
    xsel = jnp.broadcast_to(xsel, (8, D)).astype(BF16)
    idx = jnp.clip(jnp.min(tmin), 0, S - 1)
    sidx = idx // SEG
    gt = _dot(xsel, wg_v[...])
    gt = gt * jax.nn.sigmoid(gt)
    up = _dot(xsel, wu_v[...])
    gu = (gt * up).astype(BF16)
    for b in range(NBLK - 2):
        out_copy(b).wait()
    y = _dot_nt(gu, wdt_v[...])
    rsel = jax.nn.sigmoid(rmax[:, 0:1])
    upd = mod_v[5, 0:1, :] * _cat([y[0:1] * rsel, zpad[0:1]], 1)
    for j in range(4):
        blk = orow[j, sidx]
        orow[j, sidx] = jnp.where(sel, blk + upd[:, j * 128:(j + 1) * 128], blk)
    out_copy(NBLK - 2, 1).wait()
    out_copy(NBLK - 1, 1).wait()
    bsel = idx // 128
    for j in range(4):
        transpose_out(bsel, j)
    out_copy(bsel).start()
    out_copy(bsel).wait()


def pallas_adaLN_cond__memory_aug_recurrent_mem_tr__moe_arch_mod__prompt_kernel(
    A_x, A_mem0, A_Wq, A_Wk, A_Wv, A_Wo, A_seg_len, B_x, B_w_r, B_w_gate, B_w_up,
    B_w_down, c, w_mod,
):
    if isinstance(A_seg_len, int):
        assert A_seg_len == SEG
    assert A_x.shape == (1, S, D) and A_Wq.shape == (D, H, DH) and A_mem0.shape == (1, M, D)
    del B_x
    any_spec = pl.BlockSpec(memory_space=pl.ANY)
    out_t = pl.pallas_call(
        _kernel,
        out_shape=jax.ShapeDtypeStruct((D, S), BF16),
        in_specs=[any_spec] * 12,
        out_specs=any_spec,
        scratch_shapes=[
            pltpu.VMEM((D, S), BF16),
            pltpu.VMEM((2, D, 8, DH), BF16),
            pltpu.VMEM((2, D, 8, DH), BF16),
            pltpu.VMEM((2, D, 8, DH), BF16),
            pltpu.VMEM((H, D, DH), BF16),
            pltpu.VMEM((D, FF), BF16),
            pltpu.VMEM((D, FF), BF16),
            pltpu.VMEM((D, FF), BF16),
            pltpu.VMEM((D, 6 * D), BF16),
            pltpu.VMEM((2, 2, D * 4 + 16, 128), jnp.uint32),
            pltpu.VMEM((2, 2, D * 4 + 16, 128), jnp.uint32),
            pltpu.VMEM((2, 2, D * 4 + 16, 128), jnp.uint32),
            pltpu.VMEM((NT + NP, D // 2, 128), jnp.uint32),
            pltpu.VMEM((NP, 4, 64, 128), jnp.uint32),
            pltpu.VMEM((4, NSEG, SEG, 128), F32),
            pltpu.VMEM((4, NSEG, SEG, 128), F32),
            pltpu.VMEM((4, NSEG, SEG, 128), F32),
            pltpu.VMEM((4, SEG, 128), F32),
            pltpu.VMEM((NSEG, 2, NP, 4, 8, 128), jnp.uint32),
            pltpu.VMEM((NSEG, NP, 8, 128), F32),
            pltpu.VMEM((2, 4, 4, NP, 8, 128), jnp.uint32),
            pltpu.VMEM((2, 4, SEG, 128), F32),
            pltpu.VMEM((NBLK, DE, 128), BF16),
            pltpu.VMEM((8, 8, DE), F32),
            pltpu.VMEM((SEG, 128), F32),
            pltpu.VMEM((SEG, 128), jnp.int32),
            pltpu.VMEM((M, D), BF16),
            pltpu.VMEM((D,), BF16),
            pltpu.VMEM((1, D), BF16),
            pltpu.SemaphoreType.DMA((len(WAIT_GROUPS),)),
        ],
        compiler_params=pltpu.CompilerParams(vmem_limit_bytes=120 * 1024 * 1024),
    )(
        A_x.reshape(S, D).T, A_mem0.reshape(M, D),
        A_Wq, A_Wk, A_Wv,
        jnp.transpose(A_Wo, (0, 2, 1)), B_w_r, B_w_gate, B_w_up, B_w_down.T,
        c, w_mod,
    )
    return out_t.T.reshape(1, S, D)
```
